```python
import os as _os
_os.environ.setdefault("JAX_PLATFORMS", "cpu")
import jax
import jax.numpy as jnp

def _softmax(x, axis=-1):
    return jax.nn.softmax(x, axis=axis)
def _gelu(x):
    return jax.nn.gelu(x, approximate=True)
def _silu(x):
    return jax.nn.silu(x)
def _sigmoid(x):
    return jax.nn.sigmoid(x)
def _layernorm(x, axis=-1, eps=1e-5):
    m = jnp.mean(x, axis=axis, keepdims=True)
    v = jnp.var(x, axis=axis, keepdims=True)
    return (x - m) / jnp.sqrt(v + eps)
def _scatter_add(tgt, idx, src, axis=0):
    return tgt.at[idx].add(src)
def _segment_sum(src, seg, n):
    return jax.ops.segment_sum(src, seg, n)
class _Rng:
    def __init__(self, key):
        self._k = key
    def _next(self):
        self._k, sub = jax.random.split(self._k)
        return sub
    def normal(self, shape):
        return jax.random.normal(self._next(), shape, dtype=jnp.bfloat16)
    def randint(self, lo, hi, shape):
        return jax.random.randint(self._next(), shape, lo, hi, dtype=jnp.int32)
    def uniform(self, shape, lo=0.0, hi=1.0):
        return jax.random.uniform(self._next(), shape, jnp.bfloat16, lo, hi)
    def permutation(self, n):
        return jax.random.permutation(self._next(), n)


kernel_name = 'standalone__gqa_softmax__near_ridge'

def setup_inputs():
    _rng = _Rng(jax.random.key(int.from_bytes(__import__("os").urandom(4), "little")))
    _w = (lambda a: (lambda t: t.astype(jnp.bfloat16) if jnp.issubdtype(t.dtype, jnp.floating) else t)(jnp.asarray(a)))
    B, Hq, Hkv, Sq, Sk, D = 8, 32, 8, 112, 2048, 128
    return {
        "q": _w((lambda *s: _rng.normal(s) * 0.4)(B, Hq, Sq, D)),
        "k": _w((lambda *s: _rng.normal(s) * 0.4)(B, Hkv, Sk, D)),
        "v": _w((lambda *s: _rng.normal(s) * 0.05)(B, Hkv, Sk, D)),
    }

def reference(q, k, v):
    B, Hq, Sq, D = q.shape
    Hkv = k.shape[1]
    rep = Hq // Hkv
    k = jnp.repeat(k, rep, axis=1)
    v = jnp.repeat(v, rep, axis=1)
    scale = D ** -0.5
    scores = jnp.einsum("bhqd,bhkd->bhqk", q, k) * scale
    p = _softmax(scores, axis=-1)
    return jnp.einsum("bhqk,bhkd->bhqd", p, v)
```

```python
import functools
import jax, jax.numpy as jnp
from jax import lax
from jax.experimental import pallas as pl
from jax.experimental.pallas import tpu as pltpu

def make(bk=512, hb=1, vmem=64):
    @jax.jit
    def f(q,k,v):
        B,Hq,Sq,D = q.shape
        _,Hkv,Sk,_ = k.shape
        M = Hq//Hkv*Sq
        G = B*Hkv
        q2 = q.reshape(G, M, D); k2 = k.reshape(G,Sk,D); v2=v.reshape(G,Sk,D)
        c = D**-0.5*1.4426950408889634
        def kern(q_ref,k_ref,v_ref,o_ref):
            for h in range(hb):
                qv = q_ref[h]
                m = None
                for j in range(Sk//bk):
                    kb = k_ref[h, j*bk:(j+1)*bk, :]
                    vb = v_ref[h, j*bk:(j+1)*bk, :]
                    s = lax.dot_general(qv, kb, (((1,),(1,)),((),())), preferred_element_type=jnp.float32)
                    mb = jnp.max(s, axis=1, keepdims=True)
                    if m is None:
                        m = mb
                        p = jnp.exp2((s-m)*c)
                        l = jnp.sum(p, axis=1, keepdims=True)
                        acc = jnp.dot(p.astype(jnp.bfloat16), vb, preferred_element_type=jnp.float32)
                    else:
                        mn = jnp.maximum(m, mb)
                        a = jnp.exp2((m-mn)*c)
                        p = jnp.exp2((s-mn)*c)
                        l = a*l + jnp.sum(p, axis=1, keepdims=True)
                        acc = a*acc + jnp.dot(p.astype(jnp.bfloat16), vb, preferred_element_type=jnp.float32)
                        m = mn
                o_ref[h] = (acc / l).astype(o_ref.dtype)
        out = pl.pallas_call(
            kern,
            grid=(G//hb,),
            in_specs=[pl.BlockSpec((hb,M,D), lambda i:(i,0,0)),
                      pl.BlockSpec((hb,Sk,D), lambda i:(i,0,0)),
                      pl.BlockSpec((hb,Sk,D), lambda i:(i,0,0))],
            out_specs=pl.BlockSpec((hb,M,D), lambda i:(i,0,0)),
            out_shape=jax.ShapeDtypeStruct((G,M,D), q.dtype),
            compiler_params=pltpu.CompilerParams(dimension_semantics=("parallel",), vmem_limit_bytes=vmem*2**20),
        )(q2,k2,v2)
        return out.reshape(B,Hq,Sq,D)
    return f


_impl = make(bk=512)

@jax.jit
def pallas_standalone__gqa_softmax__near_ridge_kernel(q: jax.Array, k: jax.Array, v: jax.Array):
    return _impl(q, k, v)
```

```python
import functools
import jax, jax.numpy as jnp
from jax import lax
from jax.experimental import pallas as pl
from jax.experimental.pallas import tpu as pltpu

def make(bk=512, hb=4, vmem=100, flags=None, dep=1, order=0, qs=0, fdep=1, fj=1, fi=-2, peel=1, noload=0):
    @jax.jit
    def f(q,k,v):
        B,Hq,Sq,D = q.shape
        _,Hkv,Sk,_ = k.shape
        M = Hq//Hkv*Sq
        G = B*Hkv
        nb = Sk//bk
        nt = bk//128
        NI = G//hb
        q2 = q.reshape(G, M, D); k2 = k.reshape(G,Sk,D); v2=v.reshape(G,Sk,D)
        c = D**-0.5*1.4426950408889634
        def sc(x):
            return x if qs else x*c

        def kern(q_hbm,k_hbm,v_hbm,o_hbm, qb,kb,vb,ob, sem, fsem):
            def in_cps(it, slot):
                return [pltpu.make_async_copy(src.at[pl.ds(it*hb,hb)], dst.at[slot], sem.at[i,slot])
                        for i,(src,dst) in enumerate(((q_hbm,qb),(k_hbm,kb),(v_hbm,vb)))]
            def fine_cps(h):
                return [pltpu.make_async_copy(src.at[h], dst.at[0,h], fsem.at[i,h])
                        for i,(src,dst) in enumerate(((q_hbm,qb),(k_hbm,kb),(v_hbm,vb)))]
            def o_cp(it, slot):
                return pltpu.make_async_copy(ob.at[slot], o_hbm.at[pl.ds(it*hb,hb)], sem.at[3,slot])

            def compute(slot, z, fine):
                qc = {}
                def getq(h):
                    if h not in qc:
                        if fine:
                            for cp in fine_cps(h): cp.wait()
                        x = qb[slot,h]
                        qc[h] = (x.astype(jnp.float32)*c).astype(jnp.bfloat16) if qs else x
                    return qc[h]
                def qk(h,j):
                    return lax.dot_general(getq(h), kb[slot,h, j*bk:(j+1)*bk, :], (((1,),(1,)),((),())), preferred_element_type=jnp.float32)
                def fin(h,acc,l):
                    l = jnp.sum(l, axis=1, keepdims=True)
                    if dep:
                        l = -l
                    r = pl.reciprocal(l, approx=True)
                    r = r*(2.0 - l*r)
                    o = acc*r
                    ob[slot,h] = o.astype(ob.dtype)
                    return o
                T = hb*nb
                s_next = qk(0,0) if order==1 else None
                pend = None; olast=None
                for t in range(T):
                    h, j = divmod(t, nb)
                    if order==0:
                        s = qk(h,j)
                        if pend is not None:
                            olast = fin(*pend); pend=None
                    else:
                        s = s_next
                        if t+1<T:
                            s_next = qk(*divmod(t+1,nb))
                    vv = vb[slot,h, j*bk:(j+1)*bk, :]
                    mb = jnp.max(s, axis=1, keepdims=True)
                    if j==0:
                        mn = mb; a=None
                    else:
                        mn = jnp.maximum(m, mb)
                        a = jnp.exp2(sc(m-mn))
                    m = mn
                    ps = [jnp.exp2(sc(s[:, i*128:(i+1)*128]-mn)) for i in range(nt)]
                    if dep:
                        ls = (a*l - ps[0]) if a is not None else -ps[0]
                        for i in range(1,nt): ls = ls - ps[i]
                        ps[-1] = jnp.maximum(ps[-1], ls)
                    else:
                        ls = (a*l + ps[0]) if a is not None else ps[0]
                        for i in range(1,nt): ls = ls + ps[i]
                    l = ls
                    if fdep and not fine and j==fj and olast is not None:
                        zz = lax.bitcast_convert_type(lax.bitcast_convert_type(olast, jnp.int32) & z, jnp.float32)
                        ps[fi] = jnp.maximum(ps[fi], zz)
                    p = jnp.concatenate(ps, axis=1).astype(jnp.bfloat16)
                    pv = jnp.dot(p, vv, preferred_element_type=jnp.float32)
                    acc = pv if a is None else a*acc + pv
                    if j==nb-1:
                        if order==0 and t+1<T:
                            pend = (h,acc,l)
                        else:
                            olast = fin(h,acc,l)

            if peel:
                for h in range(hb):
                    for cp in fine_cps(h): cp.start()
                for cp in in_cps(1,1): cp.start()
                compute(0, None, True)
            else:
                for cp in in_cps(0,0): cp.start()

            def body(it, _):
                slot = lax.rem(it,2)
                @pl.when(it+1<NI)
                def _():
                    for cp in in_cps(it+1,1-slot): cp.start()
                @pl.when(it>=1)
                def _():
                    o_cp(it-1,1-slot).start()
                @pl.when(it>=2)
                def _():
                    o_cp(it-2, slot).wait()
                for cp in in_cps(it,slot): cp.wait()
                compute(slot, lax.shift_right_arithmetic(it,20), False)
            lax.fori_loop(1 if peel else 0, NI, body, None)
            o_cp(NI-1,(NI-1)%2).start()
            o_cp(NI-2,(NI-2)%2).wait()
            o_cp(NI-1,(NI-1)%2).wait()
        out = pl.pallas_call(
            kern,
            in_specs=[pl.BlockSpec(memory_space=pl.ANY)]*3,
            out_specs=pl.BlockSpec(memory_space=pl.ANY),
            out_shape=jax.ShapeDtypeStruct((G,M,D), q.dtype),
            scratch_shapes=[pltpu.VMEM((2,hb,M,D),q.dtype), pltpu.VMEM((2,hb,Sk,D),k.dtype), pltpu.VMEM((2,hb,Sk,D),v.dtype), pltpu.VMEM((2,hb,M,D),q.dtype),
                            pltpu.SemaphoreType.DMA((4,2)), pltpu.SemaphoreType.DMA((3,hb))],
            compiler_params=pltpu.CompilerParams(vmem_limit_bytes=vmem*2**20, flags=flags),
        )(q2,k2,v2)
        return out.reshape(B,Hq,Sq,D)
    return f


_impl = make(hb=4)

@jax.jit
def pallas_standalone__gqa_softmax__near_ridge_kernel(q: jax.Array, k: jax.Array, v: jax.Array):
    return _impl(q, k, v)
```

```python
import functools
import jax, jax.numpy as jnp
from jax import lax
from jax.experimental import pallas as pl
from jax.experimental.pallas import tpu as pltpu

def make(bk=512, hb=4, vmem=100, flags=None, dep=1, order=0, qs=0, fdep=1, fj=1, fi=-2, peel=1, tail1=0, two=0, nobc=1, di=-1, lastdep=1, mo=0):
    @jax.jit
    def f(q,k,v):
        B,Hq,Sq,D = q.shape
        _,Hkv,Sk,_ = k.shape
        M = Hq//Hkv*Sq
        G = B*Hkv
        nb = Sk//bk
        nt = bk//128
        NI = G//hb
        q2 = q.reshape(G, M, D); k2 = k.reshape(G,Sk,D); v2=v.reshape(G,Sk,D)
        c = D**-0.5*1.4426950408889634
        def sc(x):
            return x if qs else x*c

        def kern(q_hbm,k_hbm,v_hbm,o_hbm, qb,kb,vb,ob, sem, fsem):
            def in_cps(it, slot):
                return [pltpu.make_async_copy(src.at[pl.ds(it*hb,hb)], dst.at[slot], sem.at[i,slot])
                        for i,(src,dst) in enumerate(((q_hbm,qb),(k_hbm,kb),(v_hbm,vb)))]
            def fine_cps(h):
                return [pltpu.make_async_copy(src.at[h], dst.at[0,h], fsem.at[i,h])
                        for i,(src,dst) in enumerate(((q_hbm,qb),(k_hbm,kb),(v_hbm,vb)))]
            def o_cp(it, slot):
                return pltpu.make_async_copy(ob.at[slot], o_hbm.at[pl.ds(it*hb,hb)], sem.at[3,slot])

            def compute(slot, z, fine):
                qc = {}
                def getq(h):
                    if h not in qc:
                        if fine:
                            for cp in fine_cps(h): cp.wait()
                        x = qb[slot,h]
                        qc[h] = (x.astype(jnp.float32)*c).astype(jnp.bfloat16) if qs else x
                    return qc[h]
                def qk(h,j):
                    return lax.dot_general(getq(h), kb[slot,h, j*bk:(j+1)*bk, :], (((1,),(1,)),((),())), preferred_element_type=jnp.float32)
                def fin(h,acc,l):
                    l = jnp.sum(l, axis=1, keepdims=True)
                    if dep:
                        l = -l
                    r = pl.reciprocal(l, approx=True)
                    r = r*(2.0 - l*r)
                    o = acc*r
                    ob[slot,h] = o.astype(ob.dtype)
                    return o
                T = hb*nb
                s_next = qk(0,0) if order==1 else None
                pend = None; olast=None
                for t in range(T):
                    h, j = divmod(t, nb)
                    if order==0:
                        s = s_next if s_next is not None else qk(h,j)
                        s_next = qk(*divmod(t+1,nb)) if (tail1 and T-1-tail1<=t<T-1) else None
                        if pend is not None:
                            olast = fin(*pend); pend=None
                    else:
                        s = s_next
                        if t+1<T:
                            s_next = qk(*divmod(t+1,nb))
                    vv = vb[slot,h, j*bk:(j+1)*bk, :]
                    mb = jnp.max(s, axis=1, keepdims=True)
                    if j==0:
                        mn = mb; a=None
                    else:
                        mn = jnp.maximum(m, mb)
                        a = jnp.exp2(sc(m-mn))
                    m = mn
                    if mo:
                        mc = mn*c
                        ps = [jnp.exp2(s[:, i*128:(i+1)*128]*c-mc) for i in range(nt)]
                    else:
                        ps = [jnp.exp2(sc(s[:, i*128:(i+1)*128]-mn)) for i in range(nt)]
                    if dep:
                        ls = (a*l - ps[0]) if a is not None else -ps[0]
                        for i in range(1,nt): ls = ls - ps[i]
                        if lastdep or t<T-1: ps[di] = jnp.maximum(ps[di], ls)
                    else:
                        ls = (a*l + ps[0]) if a is not None else ps[0]
                        for i in range(1,nt): ls = ls + ps[i]
                    l = ls
                    if fdep and not fine and j==fj and olast is not None:
                        zz = lax.bitcast_convert_type(lax.bitcast_convert_type(olast, jnp.int32) & z, jnp.float32)
                        ps[fi] = jnp.maximum(ps[fi], zz)
                    p = jnp.concatenate(ps, axis=1).astype(jnp.bfloat16)
                    pv = jnp.dot(p, vv, preferred_element_type=jnp.float32)
                    acc = pv if a is None else a*acc + pv
                    if j==nb-1:
                        if order==0 and t+1<T:
                            pend = (h,acc,l)
                        else:
                            olast = fin(h,acc,l)

            if peel:
                for h in range(hb):
                    for cp in fine_cps(h): cp.start()
                for cp in in_cps(1,1): cp.start()
                compute(0, None, True)
            else:
                for cp in in_cps(0,0): cp.start()

            def body(it, _):
                slot = it & 1
                @pl.when(it+1<NI)
                def _():
                    for cp in in_cps(it+1,1-slot): cp.start()
                @pl.when(it>=1)
                def _():
                    o_cp(it-1,1-slot).start()
                @pl.when(it>=2)
                def _():
                    o_cp(it-2, slot).wait()
                for cp in in_cps(it,slot): cp.wait()
                compute(slot, lax.shift_right_arithmetic(it,20), False)
            lax.fori_loop(1 if peel else 0, NI, body, None)
            o_cp(NI-1,(NI-1)%2).start()
            o_cp(NI-2,(NI-2)%2).wait()
            o_cp(NI-1,(NI-1)%2).wait()
        out = pl.pallas_call(
            kern,
            in_specs=[pl.BlockSpec(memory_space=pl.ANY)]*3,
            out_specs=pl.BlockSpec(memory_space=pl.ANY),
            out_shape=jax.ShapeDtypeStruct((G,M,D), q.dtype),
            scratch_shapes=[pltpu.VMEM((2,hb,M,D),q.dtype), pltpu.VMEM((2,hb,Sk,D),k.dtype), pltpu.VMEM((2,hb,Sk,D),v.dtype), pltpu.VMEM((2,hb,M,D),q.dtype),
                            pltpu.SemaphoreType.DMA((4,2)), pltpu.SemaphoreType.DMA((3,hb))],
            compiler_params=pltpu.CompilerParams(vmem_limit_bytes=vmem*2**20, flags=flags, disable_bounds_checks=bool(nobc)),
        )(q2,k2,v2)
        return out.reshape(B,Hq,Sq,D)
    return f


_impl = make(hb=4, qs=1, fj=0)

@jax.jit
def pallas_standalone__gqa_softmax__near_ridge_kernel(q: jax.Array, k: jax.Array, v: jax.Array):
    return _impl(q, k, v)
```
